```python
import os as _os
_os.environ.setdefault("JAX_PLATFORMS", "cpu")
import jax
import jax.numpy as jnp

def _softmax(x, axis=-1):
    return jax.nn.softmax(x, axis=axis)
def _gelu(x):
    return jax.nn.gelu(x, approximate=True)
def _silu(x):
    return jax.nn.silu(x)
def _sigmoid(x):
    return jax.nn.sigmoid(x)
def _layernorm(x, axis=-1, eps=1e-5):
    m = jnp.mean(x, axis=axis, keepdims=True)
    v = jnp.var(x, axis=axis, keepdims=True)
    return (x - m) / jnp.sqrt(v + eps)
def _scatter_add(tgt, idx, src, axis=0):
    return tgt.at[idx].add(src)
def _segment_sum(src, seg, n):
    return jax.ops.segment_sum(src, seg, n)
class _Rng:
    def __init__(self, key):
        self._k = key
    def _next(self):
        self._k, sub = jax.random.split(self._k)
        return sub
    def normal(self, shape):
        return jax.random.normal(self._next(), shape, dtype=jnp.bfloat16)
    def randint(self, lo, hi, shape):
        return jax.random.randint(self._next(), shape, lo, hi, dtype=jnp.int32)
    def uniform(self, shape, lo=0.0, hi=1.0):
        return jax.random.uniform(self._next(), shape, jnp.bfloat16, lo, hi)
    def permutation(self, n):
        return jax.random.permutation(self._next(), n)


kernel_name = 'interleave_layers__mha_block__dense_activation_mish__prompt'

def setup_inputs():
    _rng = _Rng(jax.random.key(int.from_bytes(__import__("os").urandom(4), "little")))
    _w = (lambda a: (lambda t: t.astype(jnp.bfloat16) if jnp.issubdtype(t.dtype, jnp.floating) else t)(jnp.asarray(a)))
    def _A_setup():
        B, S, D, H = 1, 2048, 512, 32
        return {
            "x": _w((lambda *s: _rng.normal(s) * 0.05)(B, S, D)),
            "wqkv": _w((lambda *s: _rng.normal(s) * 0.05)(D, 3 * D)),
            "wo": _w((lambda *s: _rng.normal(s) * 0.05)(D, D)),
        }
    _A_in = _A_setup()

    def _B_setup():
        B, S, D, F = 1, 2048, 512, 1792
        return {
            "x": _w((lambda *s: _rng.normal(s) * 0.05)(B, S, D)),
            "w1": _w((lambda *s: _rng.normal(s) * 0.4)(D, F) * (D ** -0.5)),
            "b1": _w((lambda *s: _rng.normal(s) * 0.4)(F)),
            "w2": _w((lambda *s: _rng.normal(s) * 0.4)(F, D) * (F ** -0.5)),
        }
    _B_in = _B_setup()

    return {
        "A_x": _A_in["x"],
        "A_wqkv": _A_in["wqkv"],
        "A_wo": _A_in["wo"],
        "B_x": _B_in["x"],
        "B_w1": _B_in["w1"],
        "B_b1": _B_in["b1"],
        "B_w2": _B_in["w2"],
    }

def reference(A_x, A_wqkv, A_wo, B_x, B_w1, B_b1, B_w2):
    def _A_ref(x, wqkv, wo):
        B, S, D = x.shape
        H = 32
        Dh = D // H
        qkv = (lambda x, *d: x.transpose(*d))((x @ wqkv).reshape(B, S, 3, H, Dh), 2, 0, 3, 1, 4)
        q, k, v = qkv[0], qkv[1], qkv[2]
        scores = jnp.einsum("bhqd,bhkd->bhqk", q, k) * (Dh ** -0.5)
        p = _softmax(scores, axis=-1)
        o = jnp.einsum("bhqk,bhkd->bhqd", p, v)
        return (lambda x, *d: x.transpose(*d))(o, 0, 2, 1, 3).reshape(B, S, D) @ wo

    def _B_ref(x, w1, b1, w2):
        h = jnp.einsum("bsd,df->bsf", x, w1) + b1
        sp = jnp.log1p(jnp.exp(-jnp.abs(h))) + jnp.where(h > 0, h, jnp.zeros_like(h))
        act = h * jnp.tanh(sp)
        return jnp.einsum("bsf,fd->bsd", act, w2)

    x = A_x
    x = x + _A_ref(_layernorm(x, axis=-1), A_wqkv, A_wo)
    x = x + _B_ref(_layernorm(x, axis=-1), B_w1, B_b1, B_w2)
    x = x + _A_ref(_layernorm(x, axis=-1), A_wqkv, A_wo)
    x = x + _B_ref(_layernorm(x, axis=-1), B_w1, B_b1, B_w2)
    return x
```

```python
import jax
import jax.numpy as jnp
from jax import lax
import jax.experimental.pallas as pl
import jax.experimental.pallas.tpu as pltpu

S = 2048
D = 512
H = 32
DH = D // H
F = 1792
EPS = 1e-5
LOG2E = 1.4426950408889634
QSCALE = (DH ** -0.5) * LOG2E

T = 512
QB = 512
KC = 128
NC = S // KC
NQB = S // QB
NU = H * NQB
UN = 2
LAG = 2
RING = 4
SETUP_AT = 12


def _b16(x):
    return pltpu.bitcast(x, jnp.bfloat16)


def _i32(x):
    return pltpu.bitcast(x, jnp.int32)


def _layernorm(x):
    m = jnp.mean(x, axis=-1, keepdims=True)
    xc = x - m
    v = jnp.mean(xc * xc, axis=-1, keepdims=True)
    return xc * lax.rsqrt(v + EPS)


def _mish(h):
    sp = jnp.log1p(jnp.exp(-jnp.abs(h))) + jnp.maximum(h, 0.0)
    return h * jnp.tanh(sp)


def _kernel(x_ref, wqkv_ref, wo_ref, w1_ref, b1_ref, w2_ref, out_ref,
            xs_ref, q_ref, k_ref, vt_ref, ot_ref, qm0_ref, qm1_ref, s_ref):
    qms = (qm0_ref, qm1_ref)

    def qkv_block(b, carry):
        r0 = pl.multiple_of(b * T, T)
        r0h = pl.multiple_of(b * (T // 2), T // 2)
        xn = _layernorm(xs_ref[pl.ds(r0, T), :]).astype(jnp.bfloat16)
        qkv = jnp.dot(xn, wqkv_ref[...], preferred_element_type=jnp.float32)
        q_ref[pl.ds(r0h, T // 2), :] = _i32((qkv[:, :D] * QSCALE).astype(jnp.bfloat16))
        k_ref[pl.ds(r0h, T // 2), :] = _i32(qkv[:, D:2 * D].astype(jnp.bfloat16))
        vt_ref[:, pl.ds(r0, T)] = _i32(qkv[:, 2 * D:].T.astype(jnp.bfloat16))
        return carry

    def q_setup(u, qm_ref):
        h, qb = u // NQB, u % NQB
        goff = pl.multiple_of((h // 8) * 128, 128)
        qoff = pl.multiple_of(qb * (QB // 2), QB // 2)
        qi = q_ref[pl.ds(qoff, QB // 2), pl.ds(goff, 128)]
        lane = lax.broadcasted_iota(jnp.int32, (8, 128), 1)
        msk = jnp.where((lane >> 4) == (h % 8), jnp.int32(-1), jnp.int32(0))
        qm_ref[...] = (qi.reshape(QB // 16, 8, 128) & msk[None]).reshape(QB // 2, 128)

    def qk_step(u, c, qm_ref, slot, mprev):
        goff = pl.multiple_of((u // NQB // 8) * 128, 128)
        kc = _b16(k_ref[pl.ds(c * (KC // 2), KC // 2), pl.ds(goff, 128)])
        s = lax.dot_general(kc, _b16(qm_ref[...]), (((1,), (1,)), ((), ())),
                            preferred_element_type=jnp.float32)
        s_ref[slot] = s
        mc = jnp.max(s.reshape(KC // 8, 8, QB), axis=0)
        mc = jnp.broadcast_to(jnp.max(mc, axis=0, keepdims=True), (8, QB))
        if mprev is None:
            return mc, jnp.ones_like(mc)
        mnew = jnp.maximum(mprev, mc)
        return mnew, jnp.exp2(mprev - mnew)

    def pv_step(u, c, slot, m, alpha, l, acc):
        hoff = pl.multiple_of((u // NQB) * (DH // 2), DH // 2)
        ps = None
        pieces = []
        for r in range(KC // 8):
            p = jnp.exp2(s_ref[slot, pl.ds(r * 8, 8), :] - m)
            ps = p if ps is None else ps + p
            pieces.append(p)
        pb = jnp.concatenate(pieces, axis=0).astype(jnp.bfloat16)
        vt = _b16(vt_ref[pl.ds(hoff, DH // 2), pl.ds(c * KC, KC)])
        o = jnp.dot(vt, pb, preferred_element_type=jnp.float32)
        if alpha is None:
            return ps, o
        l = l * alpha + ps
        acc = (acc.reshape(DH // 8, 8, QB) * alpha[None]).reshape(DH, QB) + o
        return l, acc

    def pv_finish(u, l, acc):
        h, qb = u // NQB, u % NQB
        hoff = pl.multiple_of(h * DH, DH)
        qoff = pl.multiple_of(qb * QB, QB)
        ot_ref[pl.ds(hoff, DH), pl.ds(qoff, QB)] = acc / jnp.sum(l, axis=0, keepdims=True)

    def attention():
        q_setup(0, qms[0])
        pend = []
        mq = None
        for tq in range(LAG):
            mq, al = qk_step(0, tq, qms[0], tq % RING, mq)
            pend.append((mq, al))

        def body(i, carry):
            pend = list(carry)
            mq = pend[-1][0]
            u0 = i * UN
            l = acc = None
            for t in range(UN * NC):
                tq = t + LAG
                uq_rel, cq = tq // NC, tq % NC
                up_rel, cp = t // NC, t % NC
                if cq == SETUP_AT:
                    q_setup(jnp.minimum(u0 + uq_rel + 1, NU - 1), qms[(uq_rel + 1) % 2])
                mq, al = qk_step(jnp.minimum(u0 + uq_rel, NU - 1), cq, qms[uq_rel % 2], tq % RING,
                                 None if cq == 0 else mq)
                pend.append((mq, al))
                m, al = pend.pop(0)
                l, acc = pv_step(u0 + up_rel, cp, t % RING, m, None if cp == 0 else al, l, acc)
                if cp == NC - 1:
                    pv_finish(u0 + up_rel, l, acc)
            return tuple(pend)

        lax.fori_loop(0, NU // UN, body, tuple(pend))

    def post_block(b, carry):
        r0 = pl.multiple_of(b * T, T)
        o = ot_ref[:, pl.ds(r0, T)].T.astype(jnp.bfloat16)
        x = xs_ref[pl.ds(r0, T), :] + jnp.dot(o, wo_ref[...], preferred_element_type=jnp.float32)
        xn = _layernorm(x).astype(jnp.bfloat16)
        h = jnp.dot(xn, w1_ref[...], preferred_element_type=jnp.float32) + b1_ref[...].astype(jnp.float32)
        a = _mish(h).astype(jnp.bfloat16)
        x = x + jnp.dot(a, w2_ref[...], preferred_element_type=jnp.float32)
        xs_ref[pl.ds(r0, T), :] = x
        out_ref[pl.ds(r0, T), :] = x.astype(out_ref.dtype)
        return carry

    def init_block(b, carry):
        r0 = pl.multiple_of(b * T, T)
        xs_ref[pl.ds(r0, T), :] = x_ref[pl.ds(r0, T), :].astype(jnp.float32)
        return carry

    def layer(_, carry):
        lax.fori_loop(0, S // T, qkv_block, 0)
        attention()
        lax.fori_loop(0, S // T, post_block, 0)
        return carry

    lax.fori_loop(0, S // T, init_block, 0)
    lax.fori_loop(0, 2, layer, 0)


@jax.jit
def pallas_interleave_layers__mha_block__dense_activation_mish__prompt_kernel(
    A_x: jax.Array,
    A_wqkv: jax.Array,
    A_wo: jax.Array,
    B_x: jax.Array,
    B_w1: jax.Array,
    B_b1: jax.Array,
    B_w2: jax.Array,
):
    del B_x
    out = pl.pallas_call(
        _kernel,
        out_shape=jax.ShapeDtypeStruct((S, D), A_x.dtype),
        scratch_shapes=[
            pltpu.VMEM((S, D), jnp.float32),
            pltpu.VMEM((S // 2, D), jnp.int32),
            pltpu.VMEM((S // 2, D), jnp.int32),
            pltpu.VMEM((D // 2, S), jnp.int32),
            pltpu.VMEM((D, S), jnp.float32),
            pltpu.VMEM((QB // 2, 128), jnp.int32),
            pltpu.VMEM((QB // 2, 128), jnp.int32),
            pltpu.VMEM((RING, KC, QB), jnp.float32),
        ],
        compiler_params=pltpu.CompilerParams(vmem_limit_bytes=100 * 2**20),
    )(A_x.reshape(S, D), A_wqkv, A_wo, B_w1, B_b1.reshape(1, F), B_w2)
    return out.reshape(1, S, D)
```

```python
import jax
import jax.numpy as jnp
from jax import lax
import jax.experimental.pallas as pl
import jax.experimental.pallas.tpu as pltpu

S = 2048
D = 512
H = 32
DH = D // H
F = 1792
EPS = 1e-5
LOG2E = 1.4426950408889634
QSCALE = (DH ** -0.5) * LOG2E

T1 = 1024
T3 = 512
TS = 128
QB = 512
KC = 128
NC = S // KC
NQB = S // QB
NU = H * NQB
UN = 16
LAG = 2
RING = 4
SETUP_AT = 12
assert UN % 2 == 0 and NU % UN == 0 and NC % RING == 0 and LAG < RING


def _b16(x):
    return pltpu.bitcast(x, jnp.bfloat16)


def _i32(x):
    return pltpu.bitcast(x, jnp.int32)


def _layernorm(x):
    m = jnp.mean(x, axis=-1, keepdims=True)
    xc = x - m
    v = jnp.mean(xc * xc, axis=-1, keepdims=True)
    return xc * lax.rsqrt(v + EPS)


def _mish(h):
    sp = jnp.log1p(jnp.exp(-jnp.abs(h))) + jnp.maximum(h, 0.0)
    return h * jnp.tanh(sp)


def _kernel(x_hbm, wqkv_hbm, wo_hbm, w1_hbm, b1_hbm, w2_hbm, out_hbm,
            x_ref, wqkv_ref, wo_ref, w1_ref, b1_ref, w2_ref, out_ref,
            xs_ref, q_ref, k_ref, vt_ref, ot_ref, qm0_ref, qm1_ref, s_ref,
            x_sem, w_sem, o_sem):
    qms = (qm0_ref, qm1_ref)

    def x_copy(b):
        r0 = pl.multiple_of(b * T1, T1)
        return pltpu.make_async_copy(x_hbm.at[pl.ds(r0, T1), :], x_ref.at[pl.ds(r0, T1), :], x_sem.at[b])

    def out_copy(b):
        r0 = pl.multiple_of(b * T3, T3)
        return pltpu.make_async_copy(out_ref.at[pl.ds(r0, T3), :], out_hbm.at[pl.ds(r0, T3), :], o_sem.at[b])

    w_copies = [
        pltpu.make_async_copy(src, dst, w_sem.at[i])
        for i, (src, dst) in enumerate(((wqkv_hbm, wqkv_ref), (wo_hbm, wo_ref), (w1_hbm, w1_ref),
                                        (b1_hbm, b1_ref), (w2_hbm, w2_ref)))
    ]

    def qkv_block(b, layer):
        @pl.when(layer == 0)
        def _():
            x_copy(b).wait()

        for j in range(T1 // TS):
            r0 = pl.multiple_of(b * T1 + j * TS, TS)
            r0h = pl.multiple_of((b * T1 + j * TS) // 2, TS // 2)
            x = jnp.where(layer == 0, x_ref[pl.ds(r0, TS), :].astype(jnp.float32), xs_ref[pl.ds(r0, TS), :])
            xs_ref[pl.ds(r0, TS), :] = x
            xn = _layernorm(x).astype(jnp.bfloat16)
            v = jnp.dot(xn, wqkv_ref[:, 2 * D:], preferred_element_type=jnp.float32)
            vt_ref[:, pl.ds(r0, TS)] = _i32(v.T.astype(jnp.bfloat16))
            q = jnp.dot(xn, wqkv_ref[:, :D], preferred_element_type=jnp.float32)
            q_ref[pl.ds(r0h, TS // 2), :] = _i32((q * QSCALE).astype(jnp.bfloat16))
            k = jnp.dot(xn, wqkv_ref[:, D:2 * D], preferred_element_type=jnp.float32)
            k_ref[pl.ds(r0h, TS // 2), :] = _i32(k.astype(jnp.bfloat16))
        return layer

    def q_setup(u, qm_ref):
        h, qb = u // NQB, u % NQB
        goff = pl.multiple_of((h // 8) * 128, 128)
        qoff = pl.multiple_of(qb * (QB // 2), QB // 2)
        qi = q_ref[pl.ds(qoff, QB // 2), pl.ds(goff, 128)]
        lane = lax.broadcasted_iota(jnp.int32, (8, 128), 1)
        msk = jnp.where((lane >> 4) == (h % 8), jnp.int32(-1), jnp.int32(0))
        qm_ref[...] = (qi.reshape(QB // 16, 8, 128) & msk[None]).reshape(QB // 2, 128)

    def qk_step(u, c, qm_ref, slot, mprev):
        goff = pl.multiple_of((u // NQB // 8) * 128, 128)
        kc = _b16(k_ref[pl.ds(c * (KC // 2), KC // 2), pl.ds(goff, 128)])
        s = lax.dot_general(kc, _b16(qm_ref[...]), (((1,), (1,)), ((), ())),
                            preferred_element_type=jnp.float32)
        s_ref[slot] = s
        mc = jnp.max(s.reshape(KC // 8, 8, QB), axis=0)
        mc = jnp.broadcast_to(jnp.max(mc, axis=0, keepdims=True), (8, QB))
        if mprev is None:
            return mc, jnp.ones_like(mc)
        mnew = jnp.maximum(mprev, mc)
        return mnew, jnp.exp2(mprev - mnew)

    def pv_step(u, c, slot, m, alpha, l, acc):
        hoff = pl.multiple_of((u // NQB) * (DH // 2), DH // 2)
        ps = None
        pieces = [None] * (KC // 8)
        for r in reversed(range(KC // 8)):
            p = jnp.exp2(s_ref[slot, pl.ds(r * 8, 8), :] - m)
            ps = p if ps is None else ps + p
            pieces[r] = p
        pb = jnp.concatenate(pieces, axis=0).astype(jnp.bfloat16)
        vt = _b16(vt_ref[pl.ds(hoff, DH // 2), pl.ds(c * KC, KC)])
        o = jnp.dot(vt, pb, preferred_element_type=jnp.float32)
        if alpha is None:
            return ps, o
        l = l * alpha + ps
        acc = (acc.reshape(DH // 8, 8, QB) * alpha[None]).reshape(DH, QB) + o
        return l, acc

    def pv_finish(u, l, acc):
        h, qb = u // NQB, u % NQB
        hoff = pl.multiple_of(h * DH, DH)
        qoff = pl.multiple_of(qb * QB, QB)
        ot_ref[pl.ds(hoff, DH), pl.ds(qoff, QB)] = acc / jnp.sum(l, axis=0, keepdims=True)

    def attention():
        q_setup(0, qms[0])
        pend = []
        mq = None
        for tq in range(LAG):
            mq, al = qk_step(0, tq, qms[0], tq % RING, mq)
            pend.append((mq, al))

        def body(i, carry):
            pend = list(carry)
            mq = pend[-1][0]
            u0 = i * UN
            l = acc = None
            for t in range(UN * NC):
                tq = t + LAG
                uq_rel, cq = tq // NC, tq % NC
                up_rel, cp = t // NC, t % NC
                if cq == SETUP_AT:
                    q_setup(jnp.minimum(u0 + uq_rel + 1, NU - 1), qms[(uq_rel + 1) % 2])
                mq, al = qk_step(jnp.minimum(u0 + uq_rel, NU - 1), cq, qms[uq_rel % 2], tq % RING,
                                 None if cq == 0 else mq)
                pend.append((mq, al))
                m, al = pend.pop(0)
                l, acc = pv_step(u0 + up_rel, cp, t % RING, m, None if cp == 0 else al, l, acc)
                if cp == NC - 1:
                    pv_finish(u0 + up_rel, l, acc)
            return tuple(pend)

        lax.fori_loop(0, NU // UN, body, tuple(pend))

    def post_block(b, layer):
        rows = [pl.multiple_of(b * T3 + j * TS, TS) for j in range(T3 // TS)]
        xs = []
        for r0 in rows:
            o = ot_ref[:, pl.ds(r0, TS)].T.astype(jnp.bfloat16)
            xs.append(xs_ref[pl.ds(r0, TS), :] + jnp.dot(o, wo_ref[...], preferred_element_type=jnp.float32))
        acts = []
        for x in xs:
            xn = _layernorm(x).astype(jnp.bfloat16)
            h = jnp.dot(xn, w1_ref[...], preferred_element_type=jnp.float32)
            acts.append(_mish(h + b1_ref[...].astype(jnp.float32).reshape(1, F)).astype(jnp.bfloat16))
        for r0, x, a in zip(rows, xs, acts):
            x = x + jnp.dot(a, w2_ref[...], preferred_element_type=jnp.float32)
            xs_ref[pl.ds(r0, TS), :] = x
            out_ref[pl.ds(r0, TS), :] = x.astype(out_ref.dtype)

        @pl.when(layer == 1)
        def _():
            out_copy(b).start()
        return layer

    def layer_fn(layer, carry):
        lax.fori_loop(0, S // T1, qkv_block, layer)

        @pl.when(layer == 0)
        def _():
            for c in w_copies[1:]:
                c.start()

        attention()

        @pl.when(layer == 0)
        def _():
            for c in w_copies[1:]:
                c.wait()

        lax.fori_loop(0, S // T3, post_block, layer)
        return carry

    x_copy(0).start()
    w_copies[0].start()
    w_copies[0].wait()
    for b in range(1, S // T1):
        x_copy(b).start()
    lax.fori_loop(0, 2, layer_fn, 0)
    for b in range(S // T3):
        out_copy(b).wait()


@jax.jit
def pallas_interleave_layers__mha_block__dense_activation_mish__prompt_kernel(
    A_x: jax.Array,
    A_wqkv: jax.Array,
    A_wo: jax.Array,
    B_x: jax.Array,
    B_w1: jax.Array,
    B_b1: jax.Array,
    B_w2: jax.Array,
):
    del B_x
    out = pl.pallas_call(
        _kernel,
        out_shape=jax.ShapeDtypeStruct((S, D), A_x.dtype),
        in_specs=[pl.BlockSpec(memory_space=pl.ANY)] * 6,
        out_specs=pl.BlockSpec(memory_space=pl.ANY),
        scratch_shapes=[
            pltpu.VMEM((S, D), A_x.dtype),
            pltpu.VMEM((D, 3 * D), A_wqkv.dtype),
            pltpu.VMEM((D, D), A_wo.dtype),
            pltpu.VMEM((D, F), B_w1.dtype),
            pltpu.VMEM((F,), B_b1.dtype),
            pltpu.VMEM((F, D), B_w2.dtype),
            pltpu.VMEM((S, D), A_x.dtype),
            pltpu.VMEM((S, D), jnp.float32),
            pltpu.VMEM((S // 2, D), jnp.int32),
            pltpu.VMEM((S // 2, D), jnp.int32),
            pltpu.VMEM((D // 2, S), jnp.int32),
            pltpu.VMEM((D, S), jnp.float32),
            pltpu.VMEM((QB // 2, 128), jnp.int32),
            pltpu.VMEM((QB // 2, 128), jnp.int32),
            pltpu.VMEM((RING, KC, QB), jnp.float32),
            pltpu.SemaphoreType.DMA((S // T1,)),
            pltpu.SemaphoreType.DMA((5,)),
            pltpu.SemaphoreType.DMA((S // T3,)),
        ],
        compiler_params=pltpu.CompilerParams(vmem_limit_bytes=100 * 2**20),
    )(A_x.reshape(S, D), A_wqkv, A_wo, B_w1, B_b1, B_w2)
    return out.reshape(1, S, D)
```
